```python
import os as _os
_os.environ.setdefault("JAX_PLATFORMS", "cpu")
import jax
import jax.numpy as jnp

def _softmax(x, axis=-1):
    return jax.nn.softmax(x, axis=axis)
def _gelu(x):
    return jax.nn.gelu(x, approximate=True)
def _silu(x):
    return jax.nn.silu(x)
def _sigmoid(x):
    return jax.nn.sigmoid(x)
def _layernorm(x, axis=-1, eps=1e-5):
    m = jnp.mean(x, axis=axis, keepdims=True)
    v = jnp.var(x, axis=axis, keepdims=True)
    return (x - m) / jnp.sqrt(v + eps)
def _scatter_add(tgt, idx, src, axis=0):
    return tgt.at[idx].add(src)
def _segment_sum(src, seg, n):
    return jax.ops.segment_sum(src, seg, n)
class _Rng:
    def __init__(self, key):
        self._k = key
    def _next(self):
        self._k, sub = jax.random.split(self._k)
        return sub
    def normal(self, shape):
        return jax.random.normal(self._next(), shape, dtype=jnp.bfloat16)
    def randint(self, lo, hi, shape):
        return jax.random.randint(self._next(), shape, lo, hi, dtype=jnp.int32)
    def uniform(self, shape, lo=0.0, hi=1.0):
        return jax.random.uniform(self._next(), shape, jnp.bfloat16, lo, hi)
    def permutation(self, n):
        return jax.random.permutation(self._next(), n)


kernel_name = 'concat_heads__sliding_block_cached__sliding_block_cached__decode'

def setup_inputs():
    _rng = _Rng(jax.random.key(int.from_bytes(__import__("os").urandom(4), "little")))
    _w = (lambda a: (lambda t: t.astype(jnp.bfloat16) if jnp.issubdtype(t.dtype, jnp.floating) else t)(jnp.asarray(a)))
    def _A_setup():
        B, Sq, D = 2, 1, 640
        Hq, Hkv, Sk, Dh = 32, 32, 4096, 128
        assert Hq % Hkv == 0, (Hq, Hkv)
        return {
            "x": _w((lambda *s: _rng.normal(s) * 0.8)(B, Sq, D)),
            "k_cache": _w((lambda *s: _rng.normal(s) * 0.8)(B, Hkv, Sk, Dh)),
            "v_cache": _w((lambda *s: _rng.normal(s) * 0.05)(B, Hkv, Sk, Dh)),
            "wq": _w((lambda *s: _rng.normal(s) * 0.8)(D, Hq * Dh) * (D ** -0.5)),
            "wo": _w((lambda *s: _rng.normal(s) * 0.05)(Hq * Dh, D) * ((Hq * Dh) ** -0.5)),
        }
    _A_in = _A_setup()

    def _B_setup():
        B, Sq, D = 2, 1, 640
        Hq, Hkv, Sk, Dh = 32, 32, 4096, 128
        assert Hq % Hkv == 0, (Hq, Hkv)
        return {
            "x": _w((lambda *s: _rng.normal(s) * 0.8)(B, Sq, D)),
            "k_cache": _w((lambda *s: _rng.normal(s) * 0.8)(B, Hkv, Sk, Dh)),
            "v_cache": _w((lambda *s: _rng.normal(s) * 0.05)(B, Hkv, Sk, Dh)),
            "wq": _w((lambda *s: _rng.normal(s) * 0.8)(D, Hq * Dh) * (D ** -0.5)),
            "wo": _w((lambda *s: _rng.normal(s) * 0.05)(Hq * Dh, D) * ((Hq * Dh) ** -0.5)),
        }
    _B_in = _B_setup()

    return {
        "A_x": _A_in["x"],
        "A_k_cache": _A_in["k_cache"],
        "A_v_cache": _A_in["v_cache"],
        "A_wq": _A_in["wq"],
        "A_wo": _A_in["wo"],
        "B_x": _B_in["x"],
        "B_k_cache": _B_in["k_cache"],
        "B_v_cache": _B_in["v_cache"],
        "B_wq": _B_in["wq"],
        "B_wo": _B_in["wo"],
    }

def reference(A_x, A_k_cache, A_v_cache, A_wq, A_wo, B_x, B_k_cache, B_v_cache, B_wq, B_wo):
    def _A_ref(x, k_cache, v_cache, wq, wo):
        B, Sq, D = x.shape
        Hq, Dh = 32, 128
        Hkv, Sk = k_cache.shape[1], k_cache.shape[2]
        W = min(4096, max(256, Sk // 4))
        rep = Hq // Hkv
        q = (lambda x, *d: x.transpose(*d))((x @ wq).reshape(B, Sq, Hq, Dh), 0, 2, 1, 3)
        k = jnp.repeat(k_cache[:, :, Sk - W:, :], rep, axis=1)
        v = jnp.repeat(v_cache[:, :, Sk - W:, :], rep, axis=1)
        scores = jnp.einsum("bhqd,bhkd->bhqk", q, k) * (Dh ** -0.5)
        p = _softmax(scores, axis=-1)
        o = jnp.einsum("bhqk,bhkd->bhqd", p, v)
        return (lambda x, *d: x.transpose(*d))(o, 0, 2, 1, 3).reshape(B, Sq, Hq * Dh) @ wo

    def _B_ref(x, k_cache, v_cache, wq, wo):
        B, Sq, D = x.shape
        Hq, Dh = 32, 128
        Hkv, Sk = k_cache.shape[1], k_cache.shape[2]
        W = min(4096, max(256, Sk // 4))
        rep = Hq // Hkv
        q = (lambda x, *d: x.transpose(*d))((x @ wq).reshape(B, Sq, Hq, Dh), 0, 2, 1, 3)
        k = jnp.repeat(k_cache[:, :, Sk - W:, :], rep, axis=1)
        v = jnp.repeat(v_cache[:, :, Sk - W:, :], rep, axis=1)
        scores = jnp.einsum("bhqd,bhkd->bhqk", q, k) * (Dh ** -0.5)
        p = _softmax(scores, axis=-1)
        o = jnp.einsum("bhqk,bhkd->bhqd", p, v)
        return (lambda x, *d: x.transpose(*d))(o, 0, 2, 1, 3).reshape(B, Sq, Hq * Dh) @ wo

    a = _A_ref(A_x, A_k_cache, A_v_cache, A_wq, A_wo)
    b = _B_ref(B_x, B_k_cache, B_v_cache, B_wq, B_wo)
    return jnp.concatenate([a, b], axis=-1)
```

```python
import jax
import jax.numpy as jnp
from jax import lax
import jax.experimental.pallas as pl
import jax.experimental.pallas.tpu as pltpu

H, DH, SK, D, B = 32, 128, 4096, 640, 2
W = min(4096, max(256, SK // 4))
SCALE = DH ** -0.5

HPC = 4
G = H // HPC
N = 2 * G
NB = 2
R = 16
RB = R // 2
KVP = 8
RR = W // KVP


def _kernel(ax, ak, av, awq, awo, bx, bk, bv, bwq, bwo, out_ref,
            xbuf, kbuf, vbuf, wqbuf, wobuf, acc_ref, sems, xsem):
    def start_refs(c, refs):
        k, v, wq, wo = refs
        g = c % G
        slot = c % NB
        col = pl.multiple_of(g * (HPC * DH), HPC * DH)
        n = [0]

        def go(src, dst, sem):
            pltpu.make_async_copy(src, dst, sem).start(priority=n[0] % 2)
            n[0] += 1

        go(wq.at[:, pl.ds(col, HPC * DH)], wqbuf.at[slot], sems.at[slot, 0])
        for arr, buf, si in ((k, kbuf, 1), (v, vbuf, 2)):
            for j in range(KVP):
                for b in range(B):
                    for hl in range(HPC):
                        go(arr.at[b, g * HPC + hl, pl.ds(SK - W + j * RR, RR), :],
                           buf.at[slot, b, hl, pl.ds(j * RR, RR)], sems.at[slot, si])
        go(wo.at[pl.ds(col, HPC * DH), :], wobuf.at[slot], sems.at[slot, 3])

    def start(c):
        @pl.when(c < G)
        def _():
            start_refs(c, (ak, av, awq, awo))

        @pl.when(jnp.logical_and(c >= G, c < N))
        def _():
            start_refs(c, (bk, bv, bwq, bwo))

    xa = pltpu.make_async_copy(ax, xbuf.at[0], xsem.at[0])
    xb = pltpu.make_async_copy(bx, xbuf.at[1], xsem.at[1])
    xa.start()
    xb.start()
    start(0)
    xa.wait()
    xb.wait()
    acc_ref[...] = jnp.zeros_like(acc_ref)

    row = lax.broadcasted_iota(jnp.int32, (R, DH), 0)
    row_s = lax.broadcasted_iota(jnp.int32, (R, W), 0)

    def wait(buf, slot, i):
        pltpu.make_async_copy(buf.at[slot], buf.at[slot], sems.at[slot, i]).wait()

    def body(c, carry):
        start(c + 1)
        br = c // G
        slot = c % NB
        x2 = xbuf[br].astype(jnp.float32)
        xrep = jnp.concatenate([jnp.broadcast_to(x2[0:1], (RB, D)),
                                jnp.broadcast_to(x2[1:2], (RB, D))], axis=0).astype(jnp.bfloat16)
        wait(wqbuf, slot, 0)
        q = jnp.dot(xrep, wqbuf[slot], preferred_element_type=jnp.float32).astype(jnp.bfloat16)
        wait(kbuf, slot, 1)
        S = jnp.zeros((R, W), jnp.float32)
        for b in range(B):
            for hl in range(HPC):
                s_u = lax.dot_general(q[:, hl * DH:(hl + 1) * DH], kbuf[slot, b, hl],
                                      (((1,), (1,)), ((), ())), preferred_element_type=jnp.float32)
                S = jnp.where(row_s == b * RB + hl, s_u, S)
        S = S * SCALE
        m = jnp.max(S, axis=-1, keepdims=True)
        e = jnp.exp(S - m)
        l = jnp.sum(e, axis=-1, keepdims=True)
        P = e.astype(jnp.bfloat16)
        wait(vbuf, slot, 2)
        O = jnp.zeros((R, DH), jnp.float32)
        for b in range(B):
            for hl in range(HPC):
                o_u = jnp.dot(P, vbuf[slot, b, hl], preferred_element_type=jnp.float32)
                O = jnp.where(row == b * RB + hl, o_u, O)
        O = (O / l).astype(jnp.bfloat16)
        wait(wobuf, slot, 3)
        parts = [jnp.where((row % RB) == hl, O, jnp.zeros_like(O)) for hl in range(HPC)]
        Ocat = jnp.concatenate(parts, axis=1)
        acc_ref[br] += jnp.dot(Ocat, wobuf[slot], preferred_element_type=jnp.float32)
        return carry

    lax.fori_loop(0, N, body, 0)
    for br in range(2):
        a = acc_ref[br]
        o0 = jnp.sum(a[0:RB], axis=0, keepdims=True)
        o1 = jnp.sum(a[RB:R], axis=0, keepdims=True)
        out_ref[:, br * D:(br + 1) * D] = jnp.concatenate([o0, o1], axis=0).astype(out_ref.dtype)


@jax.jit
def pallas_concat_heads__sliding_block_cached__sliding_block_cached__decode_kernel(
    A_x: jax.Array,
    A_k_cache: jax.Array,
    A_v_cache: jax.Array,
    A_wq: jax.Array,
    A_wo: jax.Array,
    B_x: jax.Array,
    B_k_cache: jax.Array,
    B_v_cache: jax.Array,
    B_wq: jax.Array,
    B_wo: jax.Array,
):
    out = pl.pallas_call(
        _kernel,
        out_shape=jax.ShapeDtypeStruct((B, 2 * D), jnp.bfloat16),
        in_specs=[pl.BlockSpec(memory_space=pl.ANY)] * 10,
        out_specs=pl.BlockSpec(memory_space=pltpu.VMEM),
        scratch_shapes=[
            pltpu.VMEM((2, B, D), jnp.bfloat16),
            pltpu.VMEM((NB, B, HPC, W, DH), jnp.bfloat16),
            pltpu.VMEM((NB, B, HPC, W, DH), jnp.bfloat16),
            pltpu.VMEM((NB, D, HPC * DH), jnp.bfloat16),
            pltpu.VMEM((NB, HPC * DH, D), jnp.bfloat16),
            pltpu.VMEM((2, R, D), jnp.float32),
            pltpu.SemaphoreType.DMA((NB, 4)),
            pltpu.SemaphoreType.DMA((2,)),
        ],
        compiler_params=pltpu.CompilerParams(vmem_limit_bytes=64 * 1024 * 1024),
    )(A_x.reshape(B, D), A_k_cache, A_v_cache, A_wq, A_wo,
      B_x.reshape(B, D), B_k_cache, B_v_cache, B_wq, B_wo)
    return out.reshape(B, 1, 2 * D)
```

```python
import jax
import jax.numpy as jnp
from jax import lax
import jax.experimental.pallas as pl
import jax.experimental.pallas.tpu as pltpu

H, DH, SK, D, B = 32, 128, 4096, 640, 2
W = min(4096, max(256, SK // 4))
SCALE = DH ** -0.5

HPC = 2
G = H // HPC
N = 2 * G
NB = 2
R = 16
RB = R // 2
CW = HPC * DH
KVP = 8
RR = W // KVP
WQP = 10
WOP = 16


def _spread(main, extra):
    out = []
    n, m = len(main), len(extra)
    ei = 0
    for i, x in enumerate(main):
        out.append(x)
        while ei < m and (ei + 1) * n <= (i + 1) * m:
            out.append(extra[ei])
            ei += 1
    return out + extra[ei:]


def _kernel(ax, ak, av, awq, awo, bx, bk, bv, bwq, bwo, out_ref,
            xbuf, kbuf, vbuf, wqbuf, wobuf, acc_ref, sems, xsem):

    def pieces(c, refs, last):
        k, v, wq, wo = refs
        g = c % G
        slot = c % NB
        col = pl.multiple_of(g * CW, CW)
        rq = D // WQP
        wq_p = [(wq.at[pl.ds(j * rq, rq), pl.ds(col, CW)],
                 wqbuf.at[slot, pl.ds(j * rq, rq)], sems.at[slot, 0]) for j in range(WQP)]
        ro = CW // WOP
        wo_p = [(wo.at[pl.ds(col + j * ro, ro), :],
                 wobuf.at[slot, pl.ds(j * ro, ro)], sems.at[slot, 3]) for j in range(WOP)]

        def kv(arr, buf, si):
            return [(arr.at[b, g * HPC + hl, pl.ds(SK - W + j * RR, RR), :],
                     buf.at[slot, b, hl, pl.ds(j * RR, RR)], sems.at[slot, si])
                    for j in range(KVP) for b in range(B) for hl in range(HPC)]

        k_p, v_p = kv(k, kbuf, 1), kv(v, vbuf, 2)
        if last:
            return _spread(k_p, wq_p) + v_p + wo_p
        main, extra = k_p + v_p, wq_p + wo_p
        step = max(len(main) // len(extra), 1)
        out = []
        wi = 0
        for i, x in enumerate(main):
            if i % step == 0 and wi < len(extra):
                out.append(extra[wi])
                wi += 1
            out.append(x)
        return out + extra[wi:]

    def issue(lst):
        for n, (src, dst, sem) in enumerate(lst):
            pltpu.make_async_copy(src, dst, sem).start(priority=n % 2)

    refs_a = (ak, av, awq, awo)
    refs_b = (bk, bv, bwq, bwo)

    def start(c):
        @pl.when(c < G)
        def _():
            issue(pieces(c, refs_a, False))

        @pl.when(jnp.logical_and(c >= G, c < N - 1))
        def _():
            issue(pieces(c, refs_b, False))

        @pl.when(c == N - 1)
        def _():
            issue(pieces(N - 1, refs_b, True))

    xa = pltpu.make_async_copy(ax, xbuf.at[0], xsem.at[0])
    xb = pltpu.make_async_copy(bx, xbuf.at[1], xsem.at[1])
    xa.start()
    xb.start()
    issue(pieces(0, refs_a, False))
    xa.wait()
    xb.wait()
    acc_ref[...] = jnp.zeros_like(acc_ref)

    row = lax.broadcasted_iota(jnp.int32, (R, DH), 0)
    row_s = lax.broadcasted_iota(jnp.int32, (R, W), 0)

    def wait(buf, slot, i):
        pltpu.make_async_copy(buf.at[slot], buf.at[slot], sems.at[slot, i]).wait()

    def body(c, carry):
        start(c + 1)
        br = c // G
        slot = c % NB
        x2 = xbuf[br].astype(jnp.float32)
        xrep = jnp.concatenate([jnp.broadcast_to(x2[0:1], (RB, D)),
                                jnp.broadcast_to(x2[1:2], (RB, D))], axis=0).astype(jnp.bfloat16)

        wait(wqbuf, slot, 0)
        q = jnp.dot(xrep, wqbuf[slot], preferred_element_type=jnp.float32).astype(jnp.bfloat16)

        wait(kbuf, slot, 1)
        S = jnp.zeros((R, W), jnp.float32)
        for b in range(B):
            for hl in range(HPC):
                s_u = lax.dot_general(q[:, hl * DH:(hl + 1) * DH], kbuf[slot, b, hl],
                                      (((1,), (1,)), ((), ())),
                                      preferred_element_type=jnp.float32)
                S = jnp.where(row_s == b * RB + hl, s_u, S)
        S = S * SCALE
        m = jnp.max(S, axis=-1, keepdims=True)
        e = jnp.exp(S - m)
        l = jnp.sum(e, axis=-1, keepdims=True)
        P = e.astype(jnp.bfloat16)

        wait(vbuf, slot, 2)
        O = jnp.zeros((R, DH), jnp.float32)
        for b in range(B):
            for hl in range(HPC):
                o_u = jnp.dot(P, vbuf[slot, b, hl], preferred_element_type=jnp.float32)
                O = jnp.where(row == b * RB + hl, o_u, O)
        O = (O / l).astype(jnp.bfloat16)

        wait(wobuf, slot, 3)
        parts = [jnp.where((row % RB) == hl, O, jnp.zeros_like(O)) for hl in range(HPC)]
        Ocat = jnp.concatenate(parts, axis=1)
        acc_ref[br] += jnp.dot(Ocat, wobuf[slot], preferred_element_type=jnp.float32)
        return carry

    lax.fori_loop(0, N, body, 0)

    for br in range(2):
        a = acc_ref[br]
        o0 = jnp.sum(a[0:RB], axis=0, keepdims=True)
        o1 = jnp.sum(a[RB:R], axis=0, keepdims=True)
        out_ref[:, br * D:(br + 1) * D] = jnp.concatenate([o0, o1], axis=0).astype(out_ref.dtype)


@jax.jit
def pallas_concat_heads__sliding_block_cached__sliding_block_cached__decode_kernel(
    A_x: jax.Array,
    A_k_cache: jax.Array,
    A_v_cache: jax.Array,
    A_wq: jax.Array,
    A_wo: jax.Array,
    B_x: jax.Array,
    B_k_cache: jax.Array,
    B_v_cache: jax.Array,
    B_wq: jax.Array,
    B_wo: jax.Array,
):
    out = pl.pallas_call(
        _kernel,
        out_shape=jax.ShapeDtypeStruct((B, 2 * D), jnp.bfloat16),
        in_specs=[pl.BlockSpec(memory_space=pl.ANY)] * 10,
        out_specs=pl.BlockSpec(memory_space=pltpu.VMEM),
        scratch_shapes=[
            pltpu.VMEM((2, B, D), jnp.bfloat16),
            pltpu.VMEM((NB, B, HPC, W, DH), jnp.bfloat16),
            pltpu.VMEM((NB, B, HPC, W, DH), jnp.bfloat16),
            pltpu.VMEM((NB, D, CW), jnp.bfloat16),
            pltpu.VMEM((NB, CW, D), jnp.bfloat16),
            pltpu.VMEM((2, R, D), jnp.float32),
            pltpu.SemaphoreType.DMA((NB, 4)),
            pltpu.SemaphoreType.DMA((2,)),
        ],
        compiler_params=pltpu.CompilerParams(vmem_limit_bytes=64 * 1024 * 1024),
    )(A_x.reshape(B, D), A_k_cache, A_v_cache, A_wq, A_wo,
      B_x.reshape(B, D), B_k_cache, B_v_cache, B_wq, B_wo)
    return out.reshape(B, 1, 2 * D)
```
